```python
import os as _os
_os.environ.setdefault("JAX_PLATFORMS", "cpu")
import jax
import jax.numpy as jnp

def _softmax(x, axis=-1):
    return jax.nn.softmax(x, axis=axis)
def _gelu(x):
    return jax.nn.gelu(x, approximate=True)
def _silu(x):
    return jax.nn.silu(x)
def _sigmoid(x):
    return jax.nn.sigmoid(x)
def _layernorm(x, axis=-1, eps=1e-5):
    m = jnp.mean(x, axis=axis, keepdims=True)
    v = jnp.var(x, axis=axis, keepdims=True)
    return (x - m) / jnp.sqrt(v + eps)
def _scatter_add(tgt, idx, src, axis=0):
    return tgt.at[idx].add(src)
def _segment_sum(src, seg, n):
    return jax.ops.segment_sum(src, seg, n)
class _Rng:
    def __init__(self, key):
        self._k = key
    def _next(self):
        self._k, sub = jax.random.split(self._k)
        return sub
    def normal(self, shape):
        return jax.random.normal(self._next(), shape, dtype=jnp.bfloat16)
    def randint(self, lo, hi, shape):
        return jax.random.randint(self._next(), shape, lo, hi, dtype=jnp.int32)
    def uniform(self, shape, lo=0.0, hi=1.0):
        return jax.random.uniform(self._next(), shape, jnp.bfloat16, lo, hi)
    def permutation(self, n):
        return jax.random.permutation(self._next(), n)


kernel_name = 'interleave_layers__sliding_local_dilated__glu_gated_reglu__prompt'

def setup_inputs():
    _rng = _Rng(jax.random.key(int.from_bytes(__import__("os").urandom(4), "little")))
    _w = (lambda a: (lambda t: t.astype(jnp.bfloat16) if jnp.issubdtype(t.dtype, jnp.floating) else t)(jnp.asarray(a)))
    def _A_setup():
        B, S, D = 1, 2048, 512
        return {
            "x": _w((lambda *s: _rng.normal(s) * 0.05)(B, S, D)),
            "wqkv": _w((lambda *s: _rng.normal(s) * 0.05)(D, 3 * D)),
            "wo": _w((lambda *s: _rng.normal(s) * 0.05)(D, D)),
        }
    _A_in = _A_setup()

    def _B_setup():
        B, S, D, F = 1, 2048, 512, 1792
        return {
            "x": _w((lambda *s: _rng.normal(s) * 0.05)(B, S, D)),
            "W_gate": _w((lambda *s: _rng.normal(s) * 0.8)(D, F) * (2.0 / D) ** 0.5),
            "W_up": _w((lambda *s: _rng.normal(s) * 0.8)(D, F) * (2.0 / D) ** 0.5),
            "W_down": _w((lambda *s: _rng.normal(s) * 0.8)(F, D) * (1.0 / F) ** 0.5),
        }
    _B_in = _B_setup()

    return {
        "A_x": _A_in["x"],
        "A_wqkv": _A_in["wqkv"],
        "A_wo": _A_in["wo"],
        "B_x": _B_in["x"],
        "B_W_gate": _B_in["W_gate"],
        "B_W_up": _B_in["W_up"],
        "B_W_down": _B_in["W_down"],
    }

def reference(A_x, A_wqkv, A_wo, B_x, B_W_gate, B_W_up, B_W_down):
    def _A_ref(x, wqkv, wo):
        B, S, D = x.shape
        H = 32; Dh = D // H
        W, dil = 8, 2
        qkv = (lambda x, *d: x.transpose(*d))((x @ wqkv).reshape(B, S, 3, H, Dh), 2, 0, 3, 1, 4)
        q, k, v = qkv[0], qkv[1], qkv[2]
        scale = Dh ** -0.5
        pos = jnp.arange(S)
        off = jnp.arange(W) * dil
        idx = pos[:, None] - off[None, :]
        mask = idx >= 0
        idx_c = jnp.where(mask, idx, 0).reshape(-1)
        kg = k[:, :, idx_c, :].reshape(B, H, S, W, Dh)
        vg = v[:, :, idx_c, :].reshape(B, H, S, W, Dh)
        logits = jnp.einsum("bhsd,bhswd->bhsw", q, kg) * scale
        logits = jnp.where(mask[None, None, :, :], logits, -1e9)
        attn = _softmax(logits, axis=-1)
        o = jnp.einsum("bhsw,bhswd->bhsd", attn, vg)
        return (lambda x, *d: x.transpose(*d))(o, 0, 2, 1, 3).reshape(B, S, D) @ wo

    def _B_ref(x, W_gate, W_up, W_down):
        gate = jnp.einsum("bsd,df->bsf", x, W_gate)
        up = jnp.einsum("bsd,df->bsf", x, W_up)
        gate = gate * (lambda x, dt: x.astype(dt))(gate > 0, gate.dtype)
        h = gate * up
        return jnp.einsum("bsf,fd->bsd", h, W_down)

    x = A_x
    x = x + _A_ref(_layernorm(x, axis=-1), A_wqkv, A_wo)
    x = x + _B_ref(_layernorm(x, axis=-1), B_W_gate, B_W_up, B_W_down)
    x = x + _A_ref(_layernorm(x, axis=-1), A_wqkv, A_wo)
    x = x + _B_ref(_layernorm(x, axis=-1), B_W_gate, B_W_up, B_W_down)
    return x
```

```python
import functools

import jax
import jax.numpy as jnp
from jax import lax
from jax.experimental import pallas as pl
from jax.experimental.pallas import tpu as pltpu

S, D, F = 2048, 512, 1792
DH, WINDOW, DILATION = 16, 8, 2
EPS = 1e-5
LOG2E = 1.4426950408889634

T = 256
Q = T // 4
NT = S // T
NI = 2 * NT
LAG = 2
HALO = 16
WO_ROWS = 64

SCHEDULE = dict(
    qkv_parts=(1, 0, 2), qkv=(3, 1, 2, 0, 5, 6, 4), qkv_late=3, qkv_late_at=(96, 97, 98),
    groups=(0, 1, 3, 2), up_inner=(1, 5, 3, 6, 0, 4, 2), up_outer=(0, 3, 4, 1, 2, 5, 6),
    down_inner=(0, 3, 2, 1, 5, 4, 6), down_outer=(1, 3, 4, 2, 5, 6, 0),
    wo_at=(4, 8, 12, 17), first_wo_at=(4, 8, 12, 17), last_wo_at=(7, 19, 31, 43),
    norm1_at=(39, 40, 41, 43, 44, 45, 50, 52, 54, 56, 59, 60, 62, 64, 64, 66),
    norm2_at=(72, 73, 74, 75, 79, 80, 81, 81, 82, 85, 86, 86, 89, 90, 90, 91),
    tail0_at=(49, 49, 51, 53, 55, 57, 59, 61, 63, 64, 65, 67, 69, 74, 76, 79),
    tail1_at=(49, 50, 51, 53, 56, 59, 65, 68, 71, 74, 77, 79, 82, 85, 88, 91),
    first_norm_at=17,
)

f32, bf16, u32 = jnp.float32, jnp.bfloat16, jnp.uint32
cat = jnp.concatenate


def _left(a11, a12, a21, a22):
    return [a11 + a22, a21 + a22, a11, a22, a11 + a12, a21 - a11, a12 - a22]


def _right(b11, b12, b21, b22):
    return [b11 + b22, b11, b12 - b22, b21 - b11, b22, b11 + b12, b21 + b22]


_TERMS = (((0, 1), (3, 1), (4, -1), (6, 1)), ((2, 1), (4, 1)), ((1, 1), (3, 1)), ((0, 1), (1, -1), (2, 1), (5, 1)))


def _block(m, o, order):
    terms = sorted(_TERMS[o], key=lambda t: order.index(t[0]))
    if terms[0][1] < 0:
        terms[0], terms[1] = terms[1], terms[0]
    acc = m[terms[0][0]]
    for i, sign in terms[1:]:
        acc = acc + m[i] if sign > 0 else acc - m[i]
    return acc


def _two_levels(rule, blk):
    outer = [[rule(blk[i][j], blk[i][j + 2], blk[i + 2][j], blk[i + 2][j + 2]) for j in range(2)] for i in range(2)]
    return [v for r in range(7) for v in rule(outer[0][0][r], outer[0][1][r], outer[1][0][r], outer[1][1][r])]


def _dot(a, b):
    return jnp.dot(a, b, preferred_element_type=f32)


def _words(x):
    return pltpu.bitcast(x, u32)


def _matrix(words):
    return pltpu.bitcast(words, bf16)


def _unpack(words):
    return [pltpu.unpack_elementwise(words, index=i, packed_dtype=bf16, unpacked_dtype=f32) for i in range(2)]


def _pack(even, odd):
    return pltpu.pack_elementwise([even, odd], packed_dtype=bf16)


def _gather_tiles(ref, index):
    return _matrix(cat([cat([ref[i] for i in row], axis=1) for row in index], axis=0))


def _tile(j):
    return slice(j * 128, (j + 1) * 128)


def _lanes(rows):
    return lax.broadcasted_iota(jnp.int32, (rows, 128), 1)


def _layernorm(x):
    mean = jnp.sum((x[0] + x[1]) + (x[2] + x[3]), axis=1, keepdims=True) * (1.0 / D)
    d = [v - mean for v in x]
    var = jnp.sum((d[0] * d[0] + d[1] * d[1]) + (d[2] * d[2] + d[3] * d[3]), axis=1, keepdims=True) * (1.0 / D)
    rstd = jnp.exp2(jnp.log(var + EPS) * (-0.5 * LOG2E))
    return [v * rstd for v in d]


def _reciprocal(x):
    r = pl.reciprocal(x, approx=True)
    return r * (2.0 - x * r)


def _run(*work):
    for gen in work:
        for _ in gen:
            pass


def _chain(*work):
    for gen in work:
        yield from gen


def _interleave(main, steps, *sides):
    for u in range(steps + 1):
        for gen, at in sides:
            for _ in range(at.count(u)):
                next(gen)
        if u < steps:
            next(main)


def _kernel(x_hbm, wqkv_hbm, wo_hbm, wg_hbm, wu_hbm, wd_hbm, out_hbm,
            x_in, wqkv_in, wo_in, mlp_in, wd_in, wo_rows,
            w_qkv, w_o, w_mlp, w_last, lhs_qkv, lhs_mlp, resid, qkv, out_buf, sem_in, sem_out):
    sched = SCHEDULE
    parts = sched["qkv_parts"]

    copies = []

    def copy(src, dst):
        copies.append(pltpu.make_async_copy(src, dst, sem_in.at[len(copies)]))
        return copies[-1]

    def copy_x(t):
        return copy(x_hbm.at[pl.ds(t * T, T)], x_in.at[pl.ds(t * T, T)])

    def copy_qkv(p, row=0, rows=D):
        return copy(wqkv_hbm.at[pl.ds(row, rows), pl.ds(p * D, D)], wqkv_in.at[p, pl.ds(row, rows)])

    def wait(*these):
        for c in these:
            c.wait()

    x_copy = {}
    head0 = [copy_qkv(parts[0], r, 128) for r in (0, 256)]
    x_copy[0] = copy_x(0)
    head1 = [copy_qkv(parts[0], r, 128) for r in (128, 384)]
    second = copy_qkv(parts[1])
    x_copy[1] = copy_x(1)
    third = copy_qkv(parts[2])
    wo_copy = copy(wo_hbm, wo_in)
    for t in range(2, LAG + 2):
        x_copy[t] = copy_x(t)
    last = [copy(w.at[:, pl.ds(3 * D, 256)], mlp_in.at[9, :, pl.ds(256 * i, 256)])
            for i, w in enumerate((wg_hbm, wu_hbm))]
    last.append(copy(wd_hbm.at[pl.ds(3 * D, 256)], wd_in))
    mlp_sem = len(copies)
    for g in range(3):
        for i, w in enumerate((wg_hbm, wu_hbm)):
            copy(w.at[:, pl.ds(g * D, D)], mlp_in.at[2 * g + i])
    for g in range(3):
        copy(wd_hbm.at[pl.ds(g * D, D)], mlp_in.at[6 + g])
    for t in range(LAG + 2, NT):
        x_copy[t] = copy_x(t)
    for c in copies:
        c.start()

    def write_out(t):
        r0 = t * T if isinstance(t, int) else pl.multiple_of(t * T, T)
        for j in range(4):
            pltpu.make_async_copy(out_buf.at[j, pl.ds(S + r0, T)], out_hbm.at[pl.ds(r0, T), pl.ds(j * 128, 128)],
                                  sem_out.at[j]).start()

    latest = [None]

    def after(v):
        if latest[0] is None:
            return v
        token = latest[0][:8, :128]
        is_nan = token != token
        token = token if v.dtype == f32 else pltpu.bitcast(token, v.dtype)
        return cat([jnp.where(is_nan, token, v[a:a + 8]) for a in range(0, v.shape[0], 8)], axis=0)

    def prepare_qkv(p, n, lo=0, hi=128):
        lane = _lanes(n)
        group = (lane // 8) % 4
        source = (lane % 8) * 16 + 4 * group + lane // 32

        def pick(vals, shift):
            acc = vals[0]
            for i in range(1, 4):
                acc = jnp.where(group == (i + shift) % 4, vals[i], acc)
            return acc

        for a in range(lo, hi, n):
            blk = []
            for r in (2 * a, 2 * a + D // 2):
                g = [jnp.take_along_axis(after(_words(wqkv_in[p, r:r + 2 * n, _tile(i)])), source, axis=1)
                     for i in range(4)]
                diag = [pltpu.roll(pick(g, -s), 8 * s, 1) if s else pick(g, 0) for s in range(4)]
                blk.append([_unpack(pick(diag, j)) for j in range(4)])
            for j in range(2):
                even, odd = [_right(blk[0][j][e], blk[0][j + 2][e], blk[1][j][e], blk[1][j + 2][e]) for e in range(2)]
                for s in range(7):
                    w_qkv[4 * (7 * p + s) + 2 * (a // 64) + j, a % 64:a % 64 + n, :] = _pack(even[s], odd[s])
            yield

    def prepare_wo():
        for c in range(4):
            for e, v in enumerate(_unpack(_words(wo_in[:, _tile(c)]))):
                wo_rows[c, e * (D // 2):(e + 1) * (D // 2), :] = v
        yield
        for j in range(4):
            first = [g * 128 + 4 * j + (e - (g < j)) % 4 for e in range(4) for g in range(4)]
            for c in range(4):
                w = cat([wo_rows[c, pl.ds((r % 2) * (D // 2) + r // 2, 8, stride=DH // 2), :] for r in first], axis=0)
                w_o[4 * j + c] = _words(after(w).astype(bf16))
            yield

    def prepare_mlp(t, load):
        for a in range(0, 64, 8):
            blk = [[_unpack(load(slice(128 * i + 2 * a, 128 * i + 2 * a + 16), j)) for j in range(4)] for i in range(4)]
            even, odd = [_two_levels(_right, [[b[e] for b in row] for row in blk]) for e in range(2)]
            for s in range(49):
                w_mlp[49 * t + s, a:a + 8, :] = _pack(even[s], odd[s])

    def prepare_last():
        def load(rows, j):
            g, u = [_words(mlp_in[9, rows, _tile(c + j // 2)]) for c in (0, 2)]
            if j % 2 == 0:
                return jnp.where(_lanes(8) < 64, g, pltpu.roll(u, 64, 1))
            return jnp.where(_lanes(8) < 64, pltpu.roll(g, 64, 1), u)
        prepare_mlp(9, load)
        for j in range(2):
            blk = [_unpack(_words(wd_in[_tile(i), _tile(j + 2 * c)])) for i in range(2) for c in range(2)]
            even, odd = [_right(*[b[e] for b in blk]) for e in range(2)]
            for s in range(7):
                w_last[2 * s + j] = _pack(even[s], odd[s])

    def store_lhs_qkv(slot, a, top, bottom):
        for j in range(2):
            even, odd = [_left(top[e][j], top[e][j + 2], bottom[e][j], bottom[e][j + 2]) for e in range(2)]
            for s in range(7):
                lhs_qkv[14 * slot + 2 * s + j, a:a + even[s].shape[0], :] = _pack(even[s], odd[s])

    def store_lhs_mlp(a, quarters):
        even, odd = [_two_levels(_left, [v[e] for v in quarters]) for e in range(2)]
        for s in range(49):
            lhs_mlp[s, a:a + even[s].shape[0], :] = _pack(even[s], odd[s])

    def normed(r, n):
        out = []
        for e in range(2):
            x = [resid[j, pl.ds(r + e, n, stride=2), :] for j in range(4)]
            out.append(_layernorm([after(x[0])] + x[1:]))
        return out

    def norm_for_qkv(r0, slot):
        for a in range(0, T // 4, 8):
            top = normed(r0 + 2 * a, 8)
            yield
            store_lhs_qkv(slot, a, top, normed(r0 + T // 2 + 2 * a, 8))
            yield

    def norm_for_mlp(r0, n=8):
        for a in range(0, Q // 2, n):
            quarters = []
            for i in range(4):
                quarters.append(normed(r0 + i * Q + 2 * a, n))
                if i == 3:
                    store_lhs_mlp(a, quarters)
                yield

    def load_x(t):
        for j in range(4):
            resid[j, t * T:(t + 1) * T, :] = x_in[t * T:(t + 1) * T, _tile(j)].astype(f32)

    def first_norm(t):
        halves = [zip(*[_unpack(_words(x_in[r:r + T // 2, _tile(j)])) for j in range(4)])
                  for r in (t * T, t * T + T // 2)]
        store_lhs_qkv((t + LAG + 1) % 2, 0, *[[_layernorm(list(v)) for v in half] for half in halves])
        load_x(t)
        yield

    def project_qkv(r0, slot, which=parts, lead=False):
        for p in which:
            m = [None] * 7
            for i, s in enumerate(sched["qkv"]):
                b = 4 * (7 * p + s)
                m[s] = _dot(_gather_tiles(lhs_qkv, [[14 * slot + 2 * s, 14 * slot + 2 * s + 1]]),
                            _gather_tiles(w_qkv, [[b, b + 1], [b + 2, b + 3]]))
                if lead:
                    latest[0] = m[s]
                if i < 6:
                    yield
            for o in range(4):
                c = _block(m, o, sched["qkv"])
                if p == 0:
                    c = c * (DH ** -0.5 * LOG2E)
                for j in range(2):
                    qkv[4 * p + 2 * (o % 2) + j, pl.ds(r0 + HALO + (o // 2) * (T // 2), T // 2), :] = c[:, _tile(j)]
            yield

    def attend(at_start, r0, r, n):
        def window(p, j, w):
            return qkv[4 * p + j, pl.ds(r0 + HALO + r - DILATION * w, n), :]

        edge = r < HALO and at_start is not False
        if edge:
            pos = lax.broadcasted_iota(jnp.int32, (n, 128), 0) + (r + jnp.where(at_start, 0, T))
        q = [window(0, j, 0) for j in range(4)]
        logits = []
        for w in range(WINDOW):
            prod = [q[j] * window(1, j, w) for j in range(4)]
            s = (prod[0] + prod[1]) + (prod[2] + prod[3])
            s = s + pltpu.roll(s, 64, 1)
            s = s + pltpu.roll(s, 32, 1)
            logits.append(jnp.where(pos >= DILATION * w, s, -1e9 * LOG2E) if edge and w else s)
        top = functools.reduce(jnp.maximum, logits)
        e = [jnp.exp2(s - top) for s in logits]
        scale = _reciprocal(functools.reduce(jnp.add, e))

        def value(j, w):
            v = window(2, j, w)
            if edge and w:
                v = jnp.where(pos >= DILATION * w, v, qkv[8 + j, pl.ds(r0 + HALO, 8), :][0:1])
            return v

        return [functools.reduce(jnp.add, [e[w] * value(j, w) for w in range(WINDOW)]) * scale for j in range(4)]

    def attention(at_start, r0):
        for a in range(0, T, WO_ROWS):
            if a == 0:
                o = [cat(v, axis=0) for v in zip(attend(at_start, r0, 0, HALO),
                                                 attend(at_start, r0, HALO, WO_ROWS - HALO))]
            else:
                o = attend(at_start, r0, a, WO_ROWS)
            y = _dot(cat(o, axis=1).astype(bf16), _gather_tiles(w_o, [range(4 * k, 4 * k + 4) for k in range(4)]))
            for j in range(4):
                resid[j, pl.ds(r0 + a, WO_ROWS), :] += y[:, _tile(j)]
            yield

    def project_up(t, out):
        inner = [None] * 7
        for r in sched["up_outer"]:
            m = [None] * 7
            for s in sched["up_inner"]:
                m[s] = latest[0] = _dot(_matrix(lhs_mlp[7 * r + s]), _matrix(w_mlp[49 * t + 7 * r + s]))
            inner[r] = [_block(m, i, sched["up_inner"]) for i in range(4)]
            yield
        out += [[None] * 4 for _ in range(4)]
        for i in range(4):
            for o in range(4):
                out[2 * (o // 2) + i // 2][2 * (o % 2) + i % 2] = _block([v[i] for v in inner], o, sched["up_outer"])

    def mlp(r0):
        hidden = [None] * 4
        for g in sched["groups"]:
            gate, up = [], []
            if g < 3:
                yield from project_up(2 * g, gate)
                yield from project_up(2 * g + 1, up)
                h = [[jnp.maximum(a, 0.0) * b for a, b in zip(ra, rb)] for ra, rb in zip(gate, up)]
                hidden[g] = [v.astype(bf16) for v in _two_levels(_left, h)]
            else:
                yield from project_up(9, gate)
                low = _lanes(Q) < 64
                h = [[jnp.maximum(jnp.where(low, row[2 * j], pltpu.roll(row[2 * j + 1], 64, 1)), 0.0)
                      * jnp.where(low, pltpu.roll(row[2 * j], 64, 1), row[2 * j + 1]) for j in range(2)]
                     for row in gate]
                ops = [_left(h[i][0], h[i][1], h[i + 2][0], h[i + 2][1]) for i in range(2)]
                hidden[3] = [cat([ops[0][s], ops[1][s]], axis=0).astype(bf16) for s in range(7)]

        inner = [None] * 7
        pending = list(range(4))
        for r in sched["down_outer"]:
            extra = [_dot(hidden[3][r], _matrix(w_last[2 * r + j])) for j in range(2)]
            m = [None] * 7
            for s in sched["down_inner"]:
                terms = [_dot(hidden[g][7 * r + s], _matrix(w_mlp[49 * (6 + g) + 7 * r + s])) for g in range(3)]
                m[s] = latest[0] = (terms[0] + terms[1]) + terms[2]
                yield
            inner[r] = [_block(m, i, sched["down_inner"]) + extra[i % 2][(i // 2) * Q:(i // 2 + 1) * Q]
                        for i in range(4)]
            for o in [o for o in pending if all(inner[k] is not None for k, _ in _TERMS[o])]:
                pending.remove(o)
                for i in range(4):
                    row, j = (2 * (o // 2) + i // 2) * Q, 2 * (o % 2) + i % 2
                    y = resid[j, pl.ds(r0 + row, Q), :] + _block([v and v[i] for v in inner], o, sched["down_outer"])
                    resid[j, pl.ds(r0 + S + row, Q), :] = y
                    out_buf[j, pl.ds(r0 + row, Q), :] = y.astype(bf16)

    def run_mlp(r0, *sides):
        latest[0] = None
        work = mlp(r0)
        _interleave(work, 98, *sides)
        _run(work)

    qkv[4:12, 0:HALO, :] = jnp.zeros((8, HALO, 128), f32)
    wait(*head0, x_copy[0])
    _run(prepare_qkv(parts[0], 64, 0, 64), first_norm(0))
    wait(*head1)
    _run(prepare_qkv(parts[0], 64, 64, 128))
    for p, needed, side, at in (
            (parts[0], [second], prepare_qkv(parts[1], 32), (0, 1, 3, 5)),
            (parts[1], [x_copy[1], third], _chain(first_norm(1), prepare_qkv(parts[2], 32)), (0, 1, 2, 4, 5)),
            (parts[2], [wo_copy], prepare_wo(), (0, 1, 2, 4, 5))):
        latest[0] = None
        wait(*needed)
        _interleave(project_qkv(0, (LAG + 1) % 2, [p], lead=True), 7, (side, at))
    for t in range(LAG):
        latest[0] = None
        wait(x_copy[t + 2])
        side = _chain(first_norm(t + 2), norm_for_mlp(0))
        steps = 1 + (T // 16 if t == LAG - 1 else 0)
        _interleave(project_qkv((t + 1) * T, (t + LAG) % 2, lead=True), 21,
                    (attention(t == 0, t * T), sched["first_wo_at"]), (side, (sched["first_norm_at"],) * steps))
    latest[0] = None
    wait(*last)
    prepare_last()

    @pl.loop(0, 9)
    def _(t):
        pltpu.make_async_copy(mlp_in.at[t], mlp_in.at[t], sem_in.at[mlp_sem + t]).wait()
        prepare_mlp(t, lambda rows, j: _words(mlp_in[t, rows, _tile(j)]))

    wait(*[x_copy[t] for t in range(LAG + 2, NT)])
    for t in range(LAG + 2, NT):
        load_x(t)

    @pl.loop(0, NI - LAG - 1)
    def _(m):
        r0 = pl.multiple_of(m * T, T)

        @pl.when(m > NT)
        def _():
            write_out(m - 1 - NT)

        projection = project_qkv(r0 + (LAG + 1) * T, m % 2)
        _interleave(projection, 21 - sched["qkv_late"], (attention(m == NT - LAG, r0 + LAG * T), sched["wo_at"]))
        run_mlp(r0, (norm_for_qkv(r0 + (LAG + 2) * T, 1 - m % 2), sched["norm1_at"]),
                (norm_for_mlp(r0 + T), sched["norm2_at"]), (projection, sched["qkv_late_at"]))

    write_out(NT - LAG - 2)
    for i, m in enumerate(range(NI - LAG - 1, NI)):
        sides = [(norm_for_mlp((m + 1) * T), sched["tail%d_at" % i])] if m + 1 < NI else []
        if i == 0:
            sides.append((attention(False, (NI - 1) * T), sched["last_wo_at"]))
        run_mlp(m * T, *sides)
        write_out(m - NT)
    for j in range(4):
        done = out_buf.at[j, pl.ds(S, S)]
        pltpu.make_async_copy(done, done, sem_out.at[j]).wait()


@jax.jit
def pallas_interleave_layers__sliding_local_dilated__glu_gated_reglu__prompt_kernel(
    A_x: jax.Array,
    A_wqkv: jax.Array,
    A_wo: jax.Array,
    B_x: jax.Array,
    B_W_gate: jax.Array,
    B_W_up: jax.Array,
    B_W_down: jax.Array,
):
    del B_x
    assert A_x.shape == (1, S, D) and B_W_gate.shape == (D, F)
    hbm = pl.BlockSpec(memory_space=pl.ANY)
    vmem = pltpu.VMEM
    out = pl.pallas_call(
        _kernel,
        in_specs=[hbm] * 6,
        out_specs=hbm,
        out_shape=jax.ShapeDtypeStruct((S, D), bf16),
        scratch_shapes=[
            vmem((S, D), bf16), vmem((3, D, D), bf16), vmem((D, D), bf16), vmem((10, D, D), bf16),
            vmem((256, D), bf16), vmem((4, D, 128), f32),
            vmem((3 * 7 * 4, 64, 128), u32), vmem((16, 64, 128), u32), vmem((10 * 49, 64, 128), u32),
            vmem((7 * 2, 64, 128), u32),
            vmem((2 * 7 * 2, T // 4, 128), u32), vmem((49, Q // 2, 128), u32),
            vmem((4, 3 * S, 128), f32), vmem((12, HALO + 2 * S + 8, 128), f32), vmem((4, 2 * S, 128), bf16),
            pltpu.SemaphoreType.DMA((NT + 19,)), pltpu.SemaphoreType.DMA((4,)),
        ],
        compiler_params=pltpu.CompilerParams(
            vmem_limit_bytes=100 * 2**20, disable_bounds_checks=True, disable_semaphore_checks=True),
    )(A_x.reshape(S, D), A_wqkv, A_wo, B_W_gate, B_W_up, B_W_down)
    return out.reshape(1, S, D)
```

```python
import functools

import jax
import jax.numpy as jnp
from jax import lax
from jax.experimental import pallas as pl
from jax.experimental.pallas import tpu as pltpu

S, D, F = 2048, 512, 1792
DH, WINDOW, DILATION = 16, 8, 2
EPS = 1e-5
LOG2E = 1.4426950408889634

T = 256
Q = T // 4
NT = S // T
NI = 2 * NT
LAG = 2
HALO = 16
WO_ROWS = 64

SCHEDULE = dict(
    qkv_parts=(2, 1, 0),
    qkv=('1023564', '3120465', '3250461'),
    qkv_late=2,
    qkv_late_at=(94, 98),
    groups=(0, 1, 3, 2),
    up_inner=('1536204', '1532604', '1563042', '5136402', '1436052', '1536042', '1536042'),
    up_outer=('0451236', '1342056', '0342165', '0341256', '0361254', '0341256', '0541236'),
    down_inner=('0321546', '0231564', '3450612', '0324516', '0315624', '0321546', '0321546'),
    down_outer=(1, 3, 4, 2, 5, 6, 0),
    wo_at=(4, 8, 12, 18),
    first_wo_at=(4, 8, 12, 16),
    last_wo_at=(5, 17, 31, 45),
    norm1_at=(36, 36, 37, 37, 44, 45, 47, 52, 54, 56, 59, 60, 62, 64, 64, 66),
    norm2_at=(70, 71, 74, 75, 80, 81, 81, 81, 85, 85, 87, 87, 89, 90, 90, 91),
    tail0_at=(53, 53, 53, 55, 57, 61, 63, 65, 69, 69, 70, 71, 71, 76, 80, 83),
    tail1_at=(54, 54, 57, 57, 61, 62, 65, 68, 70, 73, 76, 77, 78, 79, 84, 85),
    first_norm_at=19,
    side0_at=(0, 1, 2, 4),
    side1_at=(0, 1, 3, 5),
    side2_at=(0, 0, 0, 0, 0),
)

f32, bf16, u32 = jnp.float32, jnp.bfloat16, jnp.uint32
cat = jnp.concatenate


def _left(a11, a12, a21, a22):
    return [a11 + a22, a21 + a22, a11, a22, a11 + a12, a21 - a11, a12 - a22]


def _right(b11, b12, b21, b22):
    return [b11 + b22, b11, b12 - b22, b21 - b11, b22, b11 + b12, b21 + b22]


_TERMS = (((0, 1), (3, 1), (4, -1), (6, 1)), ((2, 1), (4, 1)), ((1, 1), (3, 1)), ((0, 1), (1, -1), (2, 1), (5, 1)))


def _block(m, o, order):
    terms = sorted(_TERMS[o], key=lambda t: order.index(t[0]))
    if terms[0][1] < 0:
        terms[0], terms[1] = terms[1], terms[0]
    acc = m[terms[0][0]]
    for i, sign in terms[1:]:
        acc = acc + m[i] if sign > 0 else acc - m[i]
    return acc


def _two_levels(rule, blk):
    outer = [[rule(blk[i][j], blk[i][j + 2], blk[i + 2][j], blk[i + 2][j + 2]) for j in range(2)] for i in range(2)]
    return [v for r in range(7) for v in rule(outer[0][0][r], outer[0][1][r], outer[1][0][r], outer[1][1][r])]


def _dot(a, b):
    return jnp.dot(a, b, preferred_element_type=f32)


def _operand(ref, index):
    words = ref.bitcast(u32)
    return pltpu.bitcast(cat([cat([words[i] for i in row], axis=1) for row in index], axis=0), bf16)


def _tile(j):
    return slice(j * 128, (j + 1) * 128)


def _lanes(rows):
    return lax.broadcasted_iota(jnp.int32, (rows, 128), 1)


def _layernorm(x):
    mean = jnp.sum((x[0] + x[1]) + (x[2] + x[3]), axis=1, keepdims=True) * (1.0 / D)
    d = [v - mean for v in x]
    var = jnp.sum((d[0] * d[0] + d[1] * d[1]) + (d[2] * d[2] + d[3] * d[3]), axis=1, keepdims=True) * (1.0 / D)
    rstd = lax.rsqrt(var + EPS)
    return [v * rstd for v in d]


def _reciprocal(x):
    r = pl.reciprocal(x, approx=True)
    return r * (2.0 - x * r)


def _run(*work):
    for gen in work:
        for _ in gen:
            pass


def _chain(*work):
    for gen in work:
        yield from gen


def _interleave(main, steps, *sides):
    for u in range(steps + 1):
        for gen, at in sides:
            for _ in range(at.count(u)):
                next(gen)
        if u < steps:
            next(main)


def _kernel(x_hbm, wqkv_hbm, wo_hbm, wg_hbm, wu_hbm, wd_hbm, out_hbm,
            x_in, wqkv_in, wo_in, mlp_in, wd_in, wo_rows,
            w_qkv, w_o, w_mlp, w_last, lhs_qkv, lhs_mlp, resid, qkv, out_buf, sem_in, sem_out):
    sched = SCHEDULE
    parts = sched["qkv_parts"]

    copies = []

    def copy(src, dst):
        copies.append(pltpu.make_async_copy(src, dst, sem_in.at[len(copies)]))
        return copies[-1]

    def copy_x(t):
        return copy(x_hbm.at[pl.ds(t * T, T)], x_in.at[pl.ds(t * T, T)])

    def wait(*these):
        for c in these:
            c.wait()

    x_copy = [copy_x(0), copy_x(1)]
    first, second, third = [copy(wqkv_hbm.at[:, pl.ds(p * D, D)], wqkv_in.at[p]) for p in parts]
    wo_copy = copy(wo_hbm, wo_in)
    x_copy += [copy_x(t) for t in range(2, NT)]
    last = [copy(w.at[:, pl.ds(3 * D, 256)], mlp_in.at[9, :, pl.ds(256 * i, 256)])
            for i, w in enumerate((wg_hbm, wu_hbm))]
    last.append(copy(wd_hbm.at[pl.ds(3 * D, 256)], wd_in))
    mlp_sem = len(copies)
    for g in range(3):
        for i, w in enumerate((wg_hbm, wu_hbm)):
            copy(w.at[:, pl.ds(g * D, D)], mlp_in.at[2 * g + i])
    for g in range(3):
        copy(wd_hbm.at[pl.ds(g * D, D)], mlp_in.at[6 + g])
    for c in copies:
        c.start()

    def write_out(r0, rows=T, tiles=range(4)):
        for j in tiles:
            pltpu.make_async_copy(out_buf.at[j, pl.ds(S + r0, rows)], out_hbm.at[pl.ds(r0, rows), pl.ds(j * 128, 128)],
                                  sem_out.at[j]).start()

    latest = [None]

    def after(v):
        if latest[0] is None:
            return v
        token = latest[0][:8, :128]
        is_nan = token != token
        token = token if v.dtype == f32 else pltpu.bitcast(token, v.dtype)
        return cat([jnp.where(is_nan, token, v[a:a + 8]) for a in range(0, v.shape[0], 8)], axis=0)

    def head_major(tiles):
        lane = _lanes(tiles[0].shape[0])
        group = (lane // 8) % 4

        def pick(vals, shift):
            acc = vals[0]
            for i in range(1, 4):
                acc = jnp.where(group == (i + shift) % 4, vals[i], acc)
            return acc

        g = [jnp.take_along_axis(v, (lane % 8) * 16 + 4 * group + lane // 32, axis=1) for v in tiles]
        diag = [pltpu.roll(pick(g, -s), 8 * s, 1) if s else pick(g, 0) for s in range(4)]
        return [pick(diag, j) for j in range(4)]

    def prepare_qkv(p, n):
        for a in range(0, D // 2, n):
            blk = [[pltpu.bitcast(v, bf16).astype(f32) for v in head_major(
                [after(pltpu.bitcast(wqkv_in[p, r:r + n, _tile(i)], u32)) for i in range(4)])] for r in (a, a + D // 2)]
            for j in range(2):
                for s, w in enumerate(_right(blk[0][j], blk[0][j + 2], blk[1][j], blk[1][j + 2])):
                    for b in range(0, n, 128):
                        w_qkv[4 * (7 * p + s) + 2 * ((a + b) // 128) + j, a % 128:a % 128 + min(n, 128), :] = (
                            w[b:b + 128].astype(bf16))
            yield

    def prepare_wo():
        pitch = DH + 1
        for c in range(4):
            for h in range(D // DH):
                wo_rows[c, pitch * h:pitch * h + DH, :] = wo_in[DH * h:DH * (h + 1), _tile(c)].astype(f32)
        yield
        for j in range(4):
            rows = [8 * g * pitch + 4 * j + (e - (g < j)) % 4 for e in range(4) for g in range(4)]
            for c in range(4):
                w = cat([wo_rows[c, pl.ds(r, 8, stride=pitch), :] for r in rows], axis=0)
                w_o[4 * j + c] = after(w).astype(bf16)
            yield

    def prepare_mlp(t, load):
        for a in range(0, 128, 16):
            blk = [[load(slice(128 * i + a, 128 * i + a + 16), j).astype(f32) for j in range(4)] for i in range(4)]
            for s, w in enumerate(_two_levels(_right, blk)):
                w_mlp[49 * t + s, a:a + 16, :] = w.astype(bf16)

    def prepare_last():
        def load(rows, j):
            g, u = [pltpu.bitcast(mlp_in[9, rows, _tile(c + j // 2)], u32) for c in (0, 2)]
            g, u = (g, pltpu.roll(u, 64, 1)) if j % 2 == 0 else (pltpu.roll(g, 64, 1), u)
            return pltpu.bitcast(jnp.where(_lanes(8) < 64, g, u), bf16)
        prepare_mlp(9, load)
        for j in range(2):
            blk = [wd_in[_tile(i), _tile(j + 2 * c)].astype(f32) for i in range(2) for c in range(2)]
            for s, w in enumerate(_right(*blk)):
                w_last[2 * s + j] = w.astype(bf16)

    def store_lhs_qkv(slot, a, top, bottom):
        for j in range(2):
            for s, v in enumerate(_left(top[j], top[j + 2], bottom[j], bottom[j + 2])):
                lhs_qkv[14 * slot + 2 * s + j, a:a + v.shape[0], :] = v.astype(bf16)

    def normed(r):
        x = [resid[j, pl.ds(r, 16), :] for j in range(4)]
        return _layernorm([after(x[0])] + x[1:])

    def norm_for_qkv(r0, slot):
        for a in range(0, T // 2, 16):
            top = normed(r0 + a)
            yield
            store_lhs_qkv(slot, a, top, normed(r0 + T // 2 + a))
            yield

    def norm_for_mlp(r0):
        for a in range(0, Q, 16):
            quarters = []
            for i in range(4):
                quarters.append(normed(r0 + i * Q + a))
                if i == 3:
                    for s, v in enumerate(_two_levels(_left, quarters)):
                        lhs_mlp[s, a:a + 16, :] = v.astype(bf16)
                yield

    def load_x(t):
        for j in range(4):
            resid[j, t * T:(t + 1) * T, :] = x_in[t * T:(t + 1) * T, _tile(j)].astype(f32)

    def first_norm(t):
        halves = [_layernorm([x_in[r:r + T // 2, _tile(j)].astype(f32) for j in range(4)])
                  for r in (t * T, t * T + T // 2)]
        store_lhs_qkv((t + LAG + 1) % 2, 0, *halves)
        load_x(t)
        yield

    def project_qkv(r0, slot, which=parts, lead=False):
        for p in which:
            m = [None] * 7
            order = [int(c) for c in sched["qkv"][parts.index(p)]]
            for i, s in enumerate(order):
                b = 4 * (7 * p + s)
                m[s] = _dot(_operand(lhs_qkv, [[14 * slot + 2 * s, 14 * slot + 2 * s + 1]]),
                            _operand(w_qkv, [[b, b + 1], [b + 2, b + 3]]))
                if lead:
                    latest[0] = m[s]
                if i < 6:
                    yield
            for o in range(4):
                c = _block(m, o, order)
                if p == 0:
                    c = c * (DH ** -0.5 * LOG2E)
                for j in range(2):
                    qkv[4 * p + 2 * (o % 2) + j, pl.ds(r0 + HALO + (o // 2) * (T // 2), T // 2), :] = c[:, _tile(j)]
            yield

    def attend(at_start, r0, r, n):
        def window(p, j, w):
            return qkv[4 * p + j, pl.ds(r0 + HALO + r - DILATION * w, n), :]

        edge = r < HALO and at_start is not False
        if edge:
            pos = lax.broadcasted_iota(jnp.int32, (n, 128), 0) + (r + jnp.where(at_start, 0, T))
        q = [window(0, j, 0) for j in range(4)]
        logits = []
        for w in range(WINDOW):
            prod = [q[j] * window(1, j, w) for j in range(4)]
            s = (prod[0] + prod[1]) + (prod[2] + prod[3])
            s = s + pltpu.roll(s, 64, 1)
            s = s + pltpu.roll(s, 32, 1)
            logits.append(jnp.where(pos >= DILATION * w, s, -1e9 * LOG2E) if edge and w else s)
        top = functools.reduce(jnp.maximum, logits)
        e = [jnp.exp2(s - top) for s in logits]
        scale = _reciprocal(functools.reduce(jnp.add, e))

        def value(j, w):
            v = window(2, j, w)
            if edge and w:
                v = jnp.where(pos >= DILATION * w, v, qkv[8 + j, pl.ds(r0 + HALO, 8), :][0:1])
            return v

        return [functools.reduce(jnp.add, [e[w] * value(j, w) for w in range(WINDOW)]) * scale for j in range(4)]

    def attention(at_start, r0):
        for a in range(0, T, WO_ROWS):
            if a == 0:
                o = [cat(v, axis=0) for v in zip(attend(at_start, r0, 0, HALO),
                                                 attend(at_start, r0, HALO, WO_ROWS - HALO))]
            else:
                o = attend(at_start, r0, a, WO_ROWS)
            y = _dot(cat(o, axis=1).astype(bf16), _operand(w_o, [range(4 * k, 4 * k + 4) for k in range(4)]))
            for j in range(4):
                resid[j, pl.ds(r0 + a, WO_ROWS), :] += y[:, _tile(j)]
            yield

    def project_up(t, out):
        order, sub_order = [[int(c) for c in sched[k][min(t, 6)]] for k in ("up_outer", "up_inner")]
        inner = [None] * 7
        for r in order:
            m = [None] * 7
            for s in sub_order:
                m[s] = latest[0] = _dot(_operand(lhs_mlp, [[7 * r + s]]), _operand(w_mlp, [[49 * t + 7 * r + s]]))
            inner[r] = [_block(m, i, sub_order) for i in range(4)]
            yield
        out += [[None] * 4 for _ in range(4)]
        for i in range(4):
            for o in range(4):
                out[2 * (o // 2) + i // 2][2 * (o % 2) + i % 2] = _block([v[i] for v in inner], o, order)

    def mlp(r0):
        hidden = [None] * 4
        for g in sched["groups"]:
            gate, up = [], []
            if g < 3:
                yield from project_up(2 * g, gate)
                yield from project_up(2 * g + 1, up)
                h = [[jnp.maximum(a, 0.0) * b for a, b in zip(ra, rb)] for ra, rb in zip(gate, up)]
                hidden[g] = [v.astype(bf16) for v in _two_levels(_left, h)]
            else:
                yield from project_up(9, gate)
                low = _lanes(Q) < 64
                h = [[jnp.maximum(jnp.where(low, row[2 * j], pltpu.roll(row[2 * j + 1], 64, 1)), 0.0)
                      * jnp.where(low, pltpu.roll(row[2 * j], 64, 1), row[2 * j + 1]) for j in range(2)]
                     for row in gate]
                ops = [_left(h[i][0], h[i][1], h[i + 2][0], h[i + 2][1]) for i in range(2)]
                hidden[3] = [cat([ops[0][s], ops[1][s]], axis=0).astype(bf16) for s in range(7)]

        inner = [None] * 7
        pending = list(range(4))
        for r in sched["down_outer"]:
            extra = [_dot(hidden[3][r], _operand(w_last, [[2 * r + j]])) for j in range(2)]
            m = [None] * 7
            sub_order = [int(c) for c in sched["down_inner"][r]]
            for s in sub_order:
                terms = [_dot(hidden[g][7 * r + s], _operand(w_mlp, [[49 * (6 + g) + 7 * r + s]]))
                         for g in range(3)]
                m[s] = latest[0] = (terms[0] + terms[1]) + terms[2]
                yield
            inner[r] = [_block(m, i, sub_order) + extra[i % 2][(i // 2) * Q:(i // 2 + 1) * Q]
                        for i in range(4)]
            for o in [o for o in pending if all(inner[k] is not None for k, _ in _TERMS[o])]:
                pending.remove(o)
                for i in range(4):
                    row, j = (2 * (o // 2) + i // 2) * Q, 2 * (o % 2) + i % 2
                    y = resid[j, pl.ds(r0 + row, Q), :] + _block([v and v[i] for v in inner], o, sched["down_outer"])
                    resid[j, pl.ds(r0 + S + row, Q), :] = y
                    out_buf[j, pl.ds(r0 + row, Q), :] = y.astype(bf16)
                if isinstance(r0, int) and r0 == (NI - 1) * T:
                    write_out(r0 - S + (o // 2) * 2 * Q, 2 * Q, (2 * (o % 2), 2 * (o % 2) + 1))

    def run_mlp(r0, *sides):
        latest[0] = None
        work = mlp(r0)
        _interleave(work, 98, *sides)
        _run(work)

    qkv[4:12, 0:HALO, :] = jnp.zeros((8, HALO, 128), f32)
    for t in range(2):
        wait(x_copy[t])
        _run(first_norm(t))
    wait(first)
    _run(prepare_qkv(parts[0], D // 2))
    for p, needed, side, at in (
            (parts[0], [second], prepare_qkv(parts[1], 64), sched["side0_at"]),
            (parts[1], [third], prepare_qkv(parts[2], 64), sched["side1_at"]),
            (parts[2], [wo_copy], prepare_wo(), sched["side2_at"])):
        latest[0] = None
        wait(*needed)
        _interleave(project_qkv(0, (LAG + 1) % 2, [p], lead=True), 7, (side, at))
    for t in range(LAG):
        latest[0] = None
        later = range(LAG + 2, NT) if t == LAG - 1 else []
        wait(x_copy[t + 2], *[x_copy[u] for u in later])
        for u in later:
            load_x(u)
        side = _chain(first_norm(t + 2), norm_for_mlp(0))
        steps = 1 + (T // 16 if t == LAG - 1 else 0)
        _interleave(project_qkv((t + 1) * T, (t + LAG) % 2, lead=True), 21,
                    (attention(t == 0, t * T), sched["first_wo_at"]), (side, (sched["first_norm_at"],) * steps))
    latest[0] = None
    wait(*last)
    prepare_last()

    @pl.loop(0, 9)
    def _(t):
        pltpu.make_async_copy(mlp_in.at[t], mlp_in.at[t], sem_in.at[mlp_sem + t]).wait()
        prepare_mlp(t, lambda rows, j: mlp_in[t, rows, _tile(j)])

    @pl.loop(0, NI - LAG - 1)
    def _(m):
        r0 = pl.multiple_of(m * T, T)

        @pl.when(m > NT)
        def _():
            write_out(pl.multiple_of(r0 - (S + T), T))

        projection = project_qkv(r0 + (LAG + 1) * T, m % 2)
        _interleave(projection, 21 - sched["qkv_late"], (attention(m == NT - LAG, r0 + LAG * T), sched["wo_at"]))
        run_mlp(r0, (norm_for_qkv(r0 + (LAG + 2) * T, 1 - m % 2), sched["norm1_at"]),
                (norm_for_mlp(r0 + T), sched["norm2_at"]), (projection, sched["qkv_late_at"]))

    write_out((NT - LAG - 2) * T)
    for i, m in enumerate(range(NI - LAG - 1, NI)):
        sides = [(norm_for_mlp((m + 1) * T), sched["tail%d_at" % i])] if m + 1 < NI else []
        if i == 0:
            sides.append((attention(False, (NI - 1) * T), sched["last_wo_at"]))
        run_mlp(m * T, *sides)
        if m + 1 < NI:
            write_out(m * T - S)
    for j in range(4):
        done = out_buf.at[j, pl.ds(S, S)]
        pltpu.make_async_copy(done, done, sem_out.at[j]).wait()


@jax.jit
def pallas_interleave_layers__sliding_local_dilated__glu_gated_reglu__prompt_kernel(
    A_x: jax.Array,
    A_wqkv: jax.Array,
    A_wo: jax.Array,
    B_x: jax.Array,
    B_W_gate: jax.Array,
    B_W_up: jax.Array,
    B_W_down: jax.Array,
):
    del B_x
    assert A_x.shape == (1, S, D) and B_W_gate.shape == (D, F)
    hbm = pl.BlockSpec(memory_space=pl.ANY)
    vmem = pltpu.VMEM
    out = pl.pallas_call(
        _kernel,
        in_specs=[hbm] * 6,
        out_specs=hbm,
        out_shape=jax.ShapeDtypeStruct((S, D), bf16),
        scratch_shapes=[
            vmem((S, D), bf16), vmem((3, D, D), bf16), vmem((D, D), bf16), vmem((10, D, D), bf16),
            vmem((256, D), bf16), vmem((4, D + 48, 128), f32),
            vmem((3 * 7 * 4, 128, 128), bf16), vmem((16, 128, 128), bf16), vmem((10 * 49, 128, 128), bf16),
            vmem((7 * 2, 128, 128), bf16),
            vmem((2 * 7 * 2, T // 2, 128), bf16), vmem((49, Q, 128), bf16),
            vmem((4, 3 * S, 128), f32), vmem((12, HALO + 2 * S + 8, 128), f32), vmem((4, 2 * S, 128), bf16),
            pltpu.SemaphoreType.DMA((NT + 16,)), pltpu.SemaphoreType.DMA((4,)),
        ],
        compiler_params=pltpu.CompilerParams(
            vmem_limit_bytes=100 * 2**20, disable_bounds_checks=True, disable_semaphore_checks=True),
    )(A_x.reshape(S, D), A_wqkv, A_wo, B_W_gate, B_W_up, B_W_down)
    return out.reshape(1, S, D)
```
